```python
import os as _os
_os.environ.setdefault('JAX_PLATFORMS', 'cpu')
import jax
import jax.numpy as jnp

def _softmax(x, axis=-1):
    return jax.nn.softmax(x, axis=axis)

def _gelu(x):
    return jax.nn.gelu(x, approximate=True)

def _silu(x):
    return jax.nn.silu(x)

def _sigmoid(x):
    return jax.nn.sigmoid(x)

def _layernorm(x, axis=-1, eps=1e-05):
    m = jnp.mean(x, axis=axis, keepdims=True)
    v = jnp.var(x, axis=axis, keepdims=True)
    return (x - m) / jnp.sqrt(v + eps)

def _scatter_add(tgt, idx, src, axis=0):
    return tgt.at[idx].add(src)

def _segment_sum(src, seg, n):
    return jax.ops.segment_sum(src, seg, n)

class _Rng:

    def __init__(self, key):
        self._k = key

    def _next(self):
        self._k, sub = jax.random.split(self._k)
        return sub

    def normal(self, shape):
        return jax.random.normal(self._next(), shape, dtype=jnp.bfloat16)

    def randint(self, lo, hi, shape):
        return jax.random.randint(self._next(), shape, lo, hi, dtype=jnp.int32)

    def uniform(self, shape, lo=0.0, hi=1.0):
        return jax.random.uniform(self._next(), shape, jnp.bfloat16, lo, hi)

    def permutation(self, n):
        return jax.random.permutation(self._next(), n)
kernel_name = 'sequential_preLN__linear_attn_block__mixer_gmlp__prompt'

def setup_inputs():
    _rng = _Rng(jax.random.key(int.from_bytes(__import__("os").urandom(4), "little")))
    _w = lambda a: (lambda t: t.astype(jnp.bfloat16) if jnp.issubdtype(t.dtype, jnp.floating) else t)(jnp.asarray(a))

    def _A_setup():
        B, S, D = (1, 2048, 512)
        return {'x': _w((lambda *s: _rng.normal(s) * 0.05)(B, S, D)), 'wqkv': _w((lambda *s: _rng.normal(s) * 0.05)(D, 3 * D)), 'wo': _w((lambda *s: _rng.normal(s) * 0.05)(D, D))}
    _A_in = _A_setup()

    def _B_setup():
        B, S, D, F = (1, 2048, 512, 1792)
        Fh = F // 2
        return {'x': _w((lambda *s: _rng.normal(s) * 0.05)(B, S, D)), 'w_in': _w((lambda *s: _rng.normal(s) * 0.4)(D, 2 * Fh)), 'w_sp': _w(0.01 * (lambda *s: _rng.normal(s) * 0.4)(S, S)), 'b_sp': _w(1.0 + 0.01 * (lambda *s: _rng.normal(s) * 0.05)(S)), 'w_out': _w((lambda *s: _rng.normal(s) * 0.05)(Fh, D))}
    _B_in = _B_setup()
    return {'A_x': _A_in['x'], 'A_wqkv': _A_in['wqkv'], 'A_wo': _A_in['wo'], 'B_x': _B_in['x'], 'B_w_in': _B_in['w_in'], 'B_w_sp': _B_in['w_sp'], 'B_b_sp': _B_in['b_sp'], 'B_w_out': _B_in['w_out']}

def reference(A_x, A_wqkv, A_wo, B_x, B_w_in, B_w_sp, B_b_sp, B_w_out):

    def _A_ref(x, wqkv, wo):
        B, S, D = x.shape
        H = 32
        Dh = D // H
        qkv = (lambda x, *d: x.transpose(*d))((x @ wqkv).reshape(B, S, 3, H, Dh), 2, 0, 3, 1, 4)
        q, k, v = (qkv[0], qkv[1], qkv[2])
        phi = lambda t: jnp.where(t > 0, t + 1, jnp.exp(t)) + 1e-06
        pq, pk = (phi(q), phi(k))
        kv = jnp.einsum('bhsd,bhse->bhde', pk, v)
        z = jnp.einsum('bhsd->bhd', pk)
        num = jnp.einsum('bhqd,bhde->bhqe', pq, kv)
        den = jnp.einsum('bhqd,bhd->bhq', pq, z)[..., None] + 1e-06
        o = num / den
        return (lambda x, *d: x.transpose(*d))(o, 0, 2, 1, 3).reshape(B, S, D) @ wo

    def _B_ref(x, w_in, w_sp, b_sp, w_out):
        B, S, D = x.shape
        F = w_in.shape[-1]
        Fh = F // 2
        z = _gelu(jnp.einsum('bsd,df->bsf', x, w_in))
        z1 = z[..., :Fh].copy()
        z2 = _layernorm(z[..., Fh:], axis=-1)
        g = jnp.einsum('ts,bsf->btf', w_sp, z2) + b_sp[None, :, None]
        return jnp.einsum('bsf,fd->bsd', z1 * g, w_out)
    x = A_x
    h = x + _A_ref(_layernorm(x, axis=-1), A_wqkv, A_wo)
    h2 = h + _B_ref(_layernorm(h, axis=-1), B_w_in, B_w_sp, B_b_sp, B_w_out)
    return h2
```

```python
import functools
import jax
import jax.numpy as jnp
from jax import lax
import jax.experimental.pallas as pl
import jax.experimental.pallas.tpu as pltpu

S, D, H, DH, FH = 2048, 512, 32, 16, 896
EPS = 1e-5
F32, BF16 = jnp.float32, jnp.bfloat16


def _ln(x, eps=EPS):
    m = jnp.mean(x, axis=-1, keepdims=True)
    xc = x - m
    v = jnp.mean(xc * xc, axis=-1, keepdims=True)
    return xc * lax.rsqrt(v + eps)


def _phi(t):
    return jnp.where(t > 0, t + 1.0, jnp.exp(t)) + 1e-6


def _gelu(x):
    return jax.nn.gelu(x, approximate=True)


def _dot(a, b):
    return jnp.dot(a, b, preferred_element_type=F32)


def make_kernel(T1, T2, T3, unroll):
    def kernel(x_hbm, wqkv_hbm, wo_hbm, win_hbm, wsp_hbm, bsp_hbm, wout_hbm, o_hbm,
               x_v, wqkv_v, wo_v, win_v, wsp_v, bsp_v, wout_v,
               pq_v, h_v, z1_v, z2_v, o_v, bias_v, sem_x, sem_w, sem_sp, sem_o):
        n1, n2, n3 = S // T1, S // T2, S // T3

        def x_copy(i):
            return pltpu.make_async_copy(x_hbm.at[0, pl.ds(i * T1, T1)], x_v.at[pl.ds(i * T1, T1)], sem_x.at[i])

        def sp_copy(i):
            return pltpu.make_async_copy(wsp_hbm.at[pl.ds(i * T3, T3)], wsp_v.at[pl.ds(i * T3, T3)], sem_sp.at[i])

        def o_copy(i):
            return pltpu.make_async_copy(o_v.at[pl.ds(i * T3, T3)], o_hbm.at[0, pl.ds(i * T3, T3)], sem_o.at[i])

        c_wqkv = pltpu.make_async_copy(wqkv_hbm, wqkv_v, sem_w.at[0])
        c_wo = pltpu.make_async_copy(wo_hbm, wo_v, sem_w.at[1])
        c_win = pltpu.make_async_copy(win_hbm, win_v, sem_w.at[2])
        c_bsp = pltpu.make_async_copy(bsp_hbm, bsp_v, sem_w.at[3])
        c_wout = pltpu.make_async_copy(wout_hbm, wout_v, sem_w.at[4])

        x_copy(0).start()
        c_wqkv.start()
        for i in range(1, n1):
            x_copy(i).start()
        c_wo.start()
        c_win.start()
        c_bsp.start()
        c_wout.start()
        for i in range(n3):
            sp_copy(i).start()

        c_wqkv.wait()

        def p1(i, carry):
            kv, z = carry
            x_copy(i).wait()
            r = pl.ds(pl.multiple_of(i * T1, T1), T1)
            xn = _ln(x_v[r, :].astype(F32)).astype(BF16)
            q = _dot(xn, wqkv_v[:, 0:D])
            pq_v[r, :] = _phi(q).astype(BF16)
            pk = _phi(_dot(xn, wqkv_v[:, D:2 * D]))
            v = _dot(xn, wqkv_v[:, 2 * D:3 * D]).astype(BF16)
            z = z + jnp.sum(pk, axis=0, keepdims=True)
            pkb = pk.astype(BF16)
            kv_new = []
            for j in range(4):
                c = slice(j * 128, (j + 1) * 128)
                kv_new.append(kv[j] + lax.dot_general(pkb[:, c], v[:, c], (((0,), (0,)), ((), ())),
                                                      preferred_element_type=F32))
            return tuple(kv_new), z

        kv0 = tuple(jnp.zeros((128, 128), F32) for _ in range(4))
        kv, z = lax.fori_loop(0, n1, p1, (kv0, jnp.zeros((1, D), F32)), unroll=unroll)

        c_wo.wait()
        c_win.wait()
        ri = lax.broadcasted_iota(jnp.int32, (128, 128), 0) // DH
        ci = lax.broadcasted_iota(jnp.int32, (128, 128), 1) // DH
        mask = ri == ci
        m_blocks, zb = [], []
        for j in range(4):
            kvm = jnp.where(mask, kv[j], 0.0).astype(BF16)
            m_blocks.append(_dot(kvm, wo_v[j * 128:(j + 1) * 128, :]).astype(BF16))
            zj = jnp.broadcast_to(z[:, j * 128:(j + 1) * 128], (128, 128)).T
            zb.append(jnp.where(mask, zj, 0.0).astype(BF16))
        mm = jnp.concatenate(m_blocks, axis=0)

        def p2(i, _):
            r = pl.ds(pl.multiple_of(i * T2, T2), T2)
            pq = pq_v[r, :]
            a = []
            for j in range(4):
                pj = pq[:, j * 128:(j + 1) * 128]
                den = _dot(pj, zb[j]) + 1e-6
                a.append((pj.astype(F32) / den).astype(BF16))
            a = jnp.concatenate(a, axis=1)
            h = x_v[r, :].astype(F32) + _dot(a, mm)
            h_v[r, :] = h
            hn = _ln(h).astype(BF16)
            z1_v[r, :] = _gelu(_dot(hn, win_v[:, 0:FH])).astype(BF16)
            z2_v[r, :] = _ln(_gelu(_dot(hn, win_v[:, FH:2 * FH]))).astype(BF16)
            return None

        lax.fori_loop(0, n2, p2, None, unroll=unroll)

        c_bsp.wait()
        c_wout.wait()
        bf = bsp_v[...].astype(F32)
        for t in range(S // 128):
            bias_v[t * 128:(t + 1) * 128, :] = jnp.broadcast_to(bf[t:t + 1, :], (128, 128)).T

        def p3(i, _):
            sp_copy(i).wait()
            r = pl.ds(pl.multiple_of(i * T3, T3), T3)
            g = _dot(wsp_v[r, :], z2_v[...])
            b = bias_v[r, :]
            b = jnp.concatenate([b] * (FH // 128), axis=1)
            y = (z1_v[r, :].astype(F32) * (g + b)).astype(BF16)
            o_v[r, :] = (h_v[r, :] + _dot(y, wout_v[...])).astype(BF16)
            o_copy(i).start()
            return None

        lax.fori_loop(0, n3, p3, None, unroll=unroll)
        for i in range(n3):
            o_copy(i).wait()

    return kernel


def build(T1=256, T2=256, T3=256, unroll=1):
    @jax.jit
    def fn(A_x, A_wqkv, A_wo, B_x, B_w_in, B_w_sp, B_b_sp, B_w_out):
        del B_x
        anyspec = pl.BlockSpec(memory_space=pl.ANY)
        return pl.pallas_call(
            make_kernel(T1, T2, T3, unroll),
            out_shape=jax.ShapeDtypeStruct((1, S, D), BF16),
            in_specs=[anyspec] * 7,
            out_specs=anyspec,
            scratch_shapes=[
                pltpu.VMEM((S, D), BF16), pltpu.VMEM((D, 3 * D), BF16), pltpu.VMEM((D, D), BF16),
                pltpu.VMEM((D, 2 * FH), BF16), pltpu.VMEM((S, S), BF16), pltpu.VMEM((S // 128, 128), BF16),
                pltpu.VMEM((FH, D), BF16),
                pltpu.VMEM((S, D), BF16), pltpu.VMEM((S, D), F32), pltpu.VMEM((S, FH), BF16),
                pltpu.VMEM((S, FH), BF16), pltpu.VMEM((S, D), BF16), pltpu.VMEM((S, 128), F32),
                pltpu.SemaphoreType.DMA((S // T1,)), pltpu.SemaphoreType.DMA((5,)),
                pltpu.SemaphoreType.DMA((S // T3,)), pltpu.SemaphoreType.DMA((S // T3,)),
            ],
            compiler_params=pltpu.CompilerParams(vmem_limit_bytes=100 * 1024 * 1024),
        )(A_x, A_wqkv, A_wo, B_w_in, B_w_sp, B_b_sp.reshape(S // 128, 128), B_w_out)
    return fn


_kernel_fn = build(**dict())


@jax.jit
def pallas_sequential_preLN__linear_attn_block__mixer_gmlp__prompt_kernel(
    A_x: jax.Array,
    A_wqkv: jax.Array,
    A_wo: jax.Array,
    B_x: jax.Array,
    B_w_in: jax.Array,
    B_w_sp: jax.Array,
    B_b_sp: jax.Array,
    B_w_out: jax.Array,
):
    return _kernel_fn(A_x, A_wqkv, A_wo, B_x, B_w_in, B_w_sp, B_b_sp, B_w_out)
```

```python
import math
import jax
import jax.numpy as jnp
from jax import lax
import jax.experimental.pallas as pl
import jax.experimental.pallas.tpu as pltpu

S, D, H, DH, FH = 2048, 512, 32, 16, 896
NH = 384
EPS = 1e-5
F32, BF16, U32 = jnp.float32, jnp.bfloat16, jnp.uint32
GC1 = math.sqrt(2.0 / math.pi)
GC2 = GC1 * 0.044715


def _ln(x, eps=EPS, scale=None):
    m = jnp.mean(x, axis=-1, keepdims=True)
    xc = x - m
    v = jnp.mean(xc * xc, axis=-1, keepdims=True)
    r = lax.rsqrt(v + eps)
    if scale is not None:
        r = r * scale
    return xc * r


def _phi(t):
    return jnp.where(t > 0, t + 1.0, jnp.exp(t)) + 1e-6


def _gelu2(x):
    u = x * (GC1 + GC2 * (x * x))
    return x + x * jnp.tanh(u)


def _recip(d):
    r = pl.reciprocal(d, approx=True)
    return r * (2.0 - d * r)


def _dotK(a, b): return jnp.dot(a, b, preferred_element_type=F32)
def _dotT(a, b): return jnp.dot(a, b, preferred_element_type=F32)
def _dotKV(a, b): return jnp.dot(a, b, preferred_element_type=F32)
def _dotM(a, b): return jnp.dot(a, b, preferred_element_type=F32)
def _dotQ(a, b): return lax.dot_general(a, b, (((1,), (1,)), ((), ())), preferred_element_type=F32)
def _dotAt(a, b): return jnp.dot(a, b, preferred_element_type=F32)
def _dotZ(a, b): return jnp.dot(a, b, preferred_element_type=F32)
def _dotG(a, b): return jnp.dot(a, b, preferred_element_type=F32)
def _dotS(a, b): return jnp.dot(a, b, preferred_element_type=F32)
def _dotO(a, b): return jnp.dot(a, b, preferred_element_type=F32)


def rows(i, T):
    if isinstance(i, int):
        return pl.ds(i * T, T)
    return pl.ds(pl.multiple_of(i * T, T), T)


def ldp(ref, i, n, c=None):
    u = ref.bitcast(U32)
    cs = range(ref.shape[0]) if c is None else [c.start // 128]
    return jnp.concatenate([pltpu.bitcast(u[c, rows(i, n // 2), :], BF16) for c in cs], axis=1)


def stp(ref, i, n, v):
    for c in range(ref.shape[0]):
        ref[c, rows(i, n), :] = v[:, c * 128:(c + 1) * 128].astype(BF16)


def lhs7(a11, a12, a21, a22):
    return (a11 + a22, a21 + a22, a11, a22, a11 + a12, a21 - a11, a12 - a22)


def rhs7(b11, b12, b21, b22):
    return (b11 + b22, b11, b12 - b22, b21 - b11, b22, b11 + b12, b21 + b22)


def strassen(M):
    m1 = M(0)
    m4 = M(3)
    x11 = m1 + m4
    m2 = M(1)
    c21 = m2 + m4
    x22 = m1 - m2
    m5 = M(4)
    x11 = x11 - m5
    m3 = M(2)
    c12 = m3 + m5
    x22 = x22 + m3
    c11 = x11 + M(6)
    c22 = x22 + M(5)
    return c11, c12, c21, c22


def head_minor_rows(ref, nc):
    return [jnp.concatenate(
        [jnp.concatenate([ref[c, pl.ds(4 * j + d, H, stride=DH), :] for d in range(4)], axis=0) for c in range(nc)],
        axis=1) for j in range(4)]


def make_kernel(T1, T2, T3, scopes, u1, u2, u3, o15, usedz, o2e):
    n1, n2, n3 = S // T1, S // T2, S // T3
    hh = T2 // 2

    def scope(name):
        return jax.named_scope(name if scopes else "k")

    def kernel(x_hbm, wqkv_hbm, wo_hbm, win_hbm, wsp_hbm, bsp_hbm, wout_hbm, o_hbm,
               x_v, wqkv_v, wo_v, win_v, wsp_v, bsp_v, wout_v,
               xn_v, h_v, bs_v, zs_v, o_v, bias_v, m_v, z1_v, pkt_v, t_v,
               wqt_v, ws_v, zrow_v, zcol_v, pa_v, pb_v, h_s, as_s, q_s, a_s, g_s,
               sem_x, sem_w, sem_sp, sem_o):

        def x_copy(i):
            return pltpu.make_async_copy(x_hbm.at[0, rows(i, T1)], x_v.at[rows(i, T1)], sem_x.at[i])

        def sp_copy(i):
            return pltpu.make_async_copy(wsp_hbm.at[rows(i, T3)], wsp_v.at[rows(i, T3)], sem_sp.at[i])

        def o_copy(i):
            return pltpu.make_async_copy(o_v.at[rows(i, T3 // 2)], o_hbm.at[0, rows(i, T3 // 2)], sem_o.at[i])

        def cols(a, b):
            return (slice(None), slice(a, b))

        c_wq = pltpu.make_async_copy(wqkv_hbm.at[cols(0, D)], wqkv_v.at[cols(0, D)], sem_w.at[0])
        c_wk = pltpu.make_async_copy(wqkv_hbm.at[cols(D, 2 * D)], wqkv_v.at[cols(D, 2 * D)], sem_w.at[1])
        c_wv = pltpu.make_async_copy(wqkv_hbm.at[cols(2 * D, 3 * D)], wqkv_v.at[cols(2 * D, 3 * D)], sem_w.at[2])
        c_wo = pltpu.make_async_copy(wo_hbm, wo_v, sem_w.at[3])
        c_win = pltpu.make_async_copy(win_hbm, win_v, sem_w.at[4])
        c_bsp = pltpu.make_async_copy(bsp_hbm, bsp_v, sem_w.at[5])
        c_wout = pltpu.make_async_copy(wout_hbm, wout_v, sem_w.at[6])

        x_copy(0).start()
        c_wk.start()
        x_copy(1).start()

        def L1(i):
            stp(xn_v, i, T1, _ln(x_v[rows(i, T1), :].astype(F32)))

        def Kp(i):
            return _dotK(ldp(xn_v, i, T1), wqkv_v[:, D:2 * D])

        def P(i, k):
            pk = _phi(k)
            stp(pkt_v.at[i], 0, D, pk.astype(BF16).T)
            return pk.reshape(T1 // 8, 8, D).sum(axis=0)

        def Tdot(i):
            return _dotT(ldp(pkt_v.at[i], 0, D), ldp(xn_v, i, T1))

        with scope("p1a"):
            x_copy(0).wait()
            L1(0)
            c_wk.wait()
            x_copy(1).wait()
            for j in range(2, n1):
                x_copy(j).start()
            k = Kp(0)
            L1(1)
            z0 = P(0, k)
            x_copy(2).wait()
            k = Kp(1)
            L1(2)
            t_v[...] = Tdot(0)
            z0 = z0 + P(1, k)
            for j in range(3, n1):
                x_copy(j).wait()
            c_wq.start()
            c_wv.start()
            c_wo.start()
            c_win.start()
            c_bsp.start()
            c_wout.start()

        def p1(i, z):
            k = Kp(i)
            L1(i + 1)
            t_v[...] += Tdot(i - 1)
            return z + P(i, k)

        with scope("p1b"):
            z = lax.fori_loop(2, n1 - 1, p1, z0, unroll=u1)

        def Q(i, b=0):
            q_s[b] = _dotQ(ldp(xn_v, i, T2), ldp(wqt_v, 0, D))

        def PA(b=0, bo=0):
            pq = _phi(q_s[b])
            w = pq * zrow_v[0:1, :]
            d = (w[:, 0:128] + w[:, 128:256]) + (w[:, 256:384] + w[:, 384:512])
            d = d + pltpu.roll(d, 64, 1)
            d = d + pltpu.roll(d, 32, 1)
            r = _recip(d + 1e-6)
            stp(a_s.at[bo], 0, T2, (pq * jnp.concatenate([r] * 4, axis=1)))

        def At(i, b=0, bo=0):
            h = x_v[rows(i, T2), :].astype(F32) + _dotAt(ldp(a_s.at[b], 0, T2), ldp(m_v, 0, D))
            h_v[rows(i, T2), :] = h
            h_s[bo] = h

        def SA(b=0, bo=0):
            hn = _ln(h_s[b])
            for k, v in enumerate(lhs7(hn[:hh, :256], hn[:hh, 256:], hn[hh:, :256], hn[hh:, 256:])):
                stp(as_s.at[bo, k], 0, hh, v)

        def SZ(i, b=0, bo=0):
            for j in range(FH // 128):
                c = slice(j * 128, (j + 1) * 128)
                c11, c12, c21, c22 = strassen(
                    lambda k: _dotZ(ldp(as_s.at[b, k], 0, hh), ldp(ws_v.at[k], 0, 256, c)))
                z1_v[rows(2 * i, hh), c] = c11
                z1_v[rows(2 * i + 1, hh), c] = c21
                g_s[bo, 0:hh, c] = _gelu2(c12)
                g_s[bo, hh:T2, c] = _gelu2(c22)

        def G2(i, b=0):
            zn = _ln(g_s[b], eps=4 * EPS, scale=0.5)
            for k, v in enumerate(rhs7(zn[:hh, 0:NH], zn[:hh, NH:2 * NH], zn[hh:, 0:NH], zn[hh:, NH:2 * NH])):
                stp(bs_v.at[k], i, hh, v)
            stp(zs_v, i, T2, zn[:, 2 * NH:])

        def ktiles(a, o):
            return jnp.concatenate([a[:, k * T2 + o * hh:k * T2 + (o + 1) * hh] for k in range(n2)], axis=1)

        def P3(t):
            Th = T3 // 2
            r1, r2 = rows(2 * t, Th), rows(2 * t + 1, Th)
            w1, w2 = wsp_v[r1, :], wsp_v[r2, :]
            a11, a12, a21, a22 = ktiles(w1, 0), ktiles(w1, 1), ktiles(w2, 0), ktiles(w2, 1)
            A7 = [v.astype(BF16) for v in lhs7(a11.astype(F32), a12.astype(F32), a21.astype(F32), a22.astype(F32))]
            A7[2], A7[3] = a11, a22
            zs = ldp(zs_v, 0, S)
            gs1, gs2 = _dotG(w1, zs), _dotG(w2, zs)
            cs = [strassen(lambda k: _dotS(A7[k], ldp(bs_v.at[k], 0, S // 2, slice(j * 128, (j + 1) * 128))))
                  for j in range(NH // 128)]
            g1 = jnp.concatenate([c[0] for c in cs] + [c[1] for c in cs] + [gs1], axis=1)
            g2 = jnp.concatenate([c[2] for c in cs] + [c[3] for c in cs] + [gs2], axis=1)
            for e, (r, g) in enumerate(((r1, g1), (r2, g2))):
                b = jnp.concatenate([bias_v[r, :]] * (FH // 128), axis=1)
                y = (_gelu2(z1_v[r, :]) * (g + b)).astype(BF16)
                o_v[r, :] = (h_v[r, :] + _dotO(y, wout_v[...])).astype(BF16)
                o_copy(2 * t + e).start()

        ri = lax.broadcasted_iota(jnp.int32, (128, 128), 0) // DH
        ci = lax.broadcasted_iota(jnp.int32, (128, 128), 1) // DH
        mask = ri == ci
        with scope("p15"):
            c_wq.wait()
            c_wv.wait()
            c_wo.wait()
            c_win.wait()
            c_bsp.wait()
            for j in range(n3):
                sp_copy(j).start()
            st = {}

            def WQP():
                for j in range(4):
                    for kb in range(4):
                        pa_v[kb, j * 128:(j + 1) * 128, :] = (
                            wqkv_v[kb * 128:(kb + 1) * 128, j * 128:(j + 1) * 128].astype(F32).T)
                for j, blk in enumerate(head_minor_rows(pa_v, 4)):
                    stp(wqt_v, j, 128, blk)

            def K7():
                st['k'] = Kp(n1 - 1)

            def T6():
                st['t'] = t_v[...] + Tdot(n1 - 2)

            def P7():
                zz = jnp.sum(z + P(n1 - 1, st['k']), axis=0, keepdims=True)
                for j in range(4):
                    zcol_v[0, j * 128:(j + 1) * 128, :] = jnp.broadcast_to(zz[:, j * 128:(j + 1) * 128], (128, 128)).T
                for j, blk in enumerate(head_minor_rows(zcol_v, 1)):
                    zrow_v[:, j * 128:(j + 1) * 128] = blk.T[0:8, :]

            def T7():
                st['tb'] = (st['t'] + Tdot(n1 - 1)).astype(BF16)

            def KV():
                tb = st['tb']
                st['kv'] = [_dotKV(tb[j * 128:(j + 1) * 128, :], wqkv_v[:, 2 * D + j * 128:2 * D + (j + 1) * 128])
                            for j in range(4)]

            def MM():
                for j in range(4):
                    kvm = jnp.where(mask, st['kv'][j], 0.0).astype(BF16)
                    mj = _dotM(kvm, wo_v[j * 128:(j + 1) * 128, :])
                    for c in range(4):
                        pb_v[c, j * 128:(j + 1) * 128, :] = mj[:, c * 128:(c + 1) * 128]
                for j, blk in enumerate(head_minor_rows(pb_v, 4)):
                    stp(m_v, j, 128, blk)

            def WS():
                f = lambda r, c: win_v[r * 256:(r + 1) * 256, c * FH:(c + 1) * FH].astype(F32)
                for k, v in enumerate(rhs7(f(0, 0), f(0, 1), f(1, 0), f(1, 1))):
                    stp(ws_v.at[k], 0, 256, v)

            def BI():
                bf = bsp_v[...].astype(F32) * 0.5
                for t in range(S // 128):
                    bias_v[t * 128:(t + 1) * 128, :] = jnp.broadcast_to(bf[t:t + 1, :], (128, 128)).T

            fs = dict(WQP=WQP, K7=K7, T6=T6, P7=P7, T7=T7, KV=KV, MM=MM, WS=WS, BI=BI,
                      Q0=lambda: Q(0, 0), Q1=lambda: Q(1, 1), Q2=lambda: Q(2, 0),
                      PA0=lambda: PA(0, 1), PA1=lambda: PA(1, 0), PA2=lambda: PA(0, 0),
                      At0=lambda: At(0, 1, 1), At1=lambda: At(1, 0, 0), SA0=lambda: SA(1, 0),
                      SZ0=lambda: SZ(0, 0, 0))
            for name in o15.split():
                fs[name]()

        def p2(i, _):
            SA()
            At(i - 1)
            Q(i)
            G2(i - 3)
            SZ(i - 2)
            PA()
            return None

        with scope("p2"):
            lax.fori_loop(3, n2, p2, None, unroll=u2)
        with scope("p2e"):
            c_wout.wait()
            for j in range(n3):
                sp_copy(j).wait()
            SA(0, 0)
            At(n2 - 1, 0, 1)
            G2(n2 - 3, 0)
            SZ(n2 - 2, 0, 1)
            SA(1, 1)
            SZ(n2 - 1, 1, 0)
            G2(n2 - 2, 1)
            G2(n2 - 1, 0)

        with scope("p3"):
            lax.fori_loop(0, n3, lambda t, _: P3(t), None, unroll=u3)
        with scope("wait_out"):
            for i in range(2 * n3):
                o_copy(i).wait()

    return kernel


ED = {'XLA_TPU_EVENLY_DISTRIBUTE_CRITICAL_NODES': True}


def build(T1=256, T2=256, T3=512, scopes=False, u1=1, u2=1, u3=1, flags=ED, usedz=False,
          o15='K7 T6 P7 T7 WQP KV Q0 MM PA0 Q1 WS PA1 Q2 At0 SA0 At1 SZ0 PA2 BI', o2e=0):
    n1, n2, n3 = S // T1, S // T2, S // T3

    @jax.jit
    def fn(A_x, A_wqkv, A_wo, B_x, B_w_in, B_w_sp, B_b_sp, B_w_out):
        del B_x
        anyspec = pl.BlockSpec(memory_space=pl.ANY)
        VM = pltpu.VMEM
        return pl.pallas_call(
            make_kernel(T1, T2, T3, scopes, u1, u2, u3, o15, usedz, o2e),
            out_shape=jax.ShapeDtypeStruct((1, S, D), BF16),
            in_specs=[anyspec] * 7,
            out_specs=anyspec,
            scratch_shapes=[
                VM((S, D), BF16), VM((D, 3 * D), BF16), VM((D, D), BF16),
                VM((D, 2 * FH), BF16), VM((S, S), BF16), VM((S // 128, 128), BF16), VM((FH, D), BF16),
                VM((4, S, 128), BF16), VM((S, D), F32), VM((7, 3, S // 2, 128), BF16),
                VM((1, S, 128), BF16), VM((S, D), BF16), VM((S, 128), F32),
                VM((4, D, 128), BF16), VM((S, FH), F32), VM((n1, T1 // 128, D, 128), BF16), VM((D, D), F32),
                VM((4, D, 128), BF16), VM((7, 7, 256, 128), BF16), VM((8, D), F32), VM((1, D, 128), F32), VM((4, D, 128), F32), VM((4, D, 128), F32),
                VM((2, T2, D), F32), VM((2, 7, 2, T2 // 2, 128), BF16), VM((2, T2, D), F32), VM((2, 4, T2, 128), BF16),
                VM((2, T2, FH), F32),
                pltpu.SemaphoreType.DMA((n1,)), pltpu.SemaphoreType.DMA((7,)),
                pltpu.SemaphoreType.DMA((n3,)), pltpu.SemaphoreType.DMA((2 * n3,)),
            ],
            compiler_params=pltpu.CompilerParams(vmem_limit_bytes=100 * 1024 * 1024, flags=flags),
        )(A_x, A_wqkv, A_wo, B_w_in, B_w_sp, B_b_sp.reshape(S // 128, 128), B_w_out)
    return fn


_kernel_fn = build(**dict())


@jax.jit
def pallas_sequential_preLN__linear_attn_block__mixer_gmlp__prompt_kernel(
    A_x: jax.Array,
    A_wqkv: jax.Array,
    A_wo: jax.Array,
    B_x: jax.Array,
    B_w_in: jax.Array,
    B_w_sp: jax.Array,
    B_b_sp: jax.Array,
    B_w_out: jax.Array,
):
    return _kernel_fn(A_x, A_wqkv, A_wo, B_x, B_w_in, B_w_sp, B_b_sp, B_w_out)
```
